```python
import jax
import jax.numpy as jnp

def _softmax(x, axis=-1):
    return jax.nn.softmax(x, axis=axis)
def _gelu(x):
    return jax.nn.gelu(x, approximate=True)
def _silu(x):
    return jax.nn.silu(x)
def _sigmoid(x):
    return jax.nn.sigmoid(x)
def _layernorm(x, axis=-1, eps=1e-5):
    m = jnp.mean(x, axis=axis, keepdims=True)
    v = jnp.var(x, axis=axis, keepdims=True)
    return (x - m) / jnp.sqrt(v + eps)
def _scatter_add(tgt, idx, src, axis=0):
    return tgt.at[idx].add(src)
def _segment_sum(src, seg, n):
    return jax.ops.segment_sum(src, seg, n)
class _Rng:
    def __init__(self, key):
        self._k = key
    def _next(self):
        self._k, sub = jax.random.split(self._k)
        return sub
    def normal(self, shape):
        return jax.random.normal(self._next(), shape, dtype=jnp.bfloat16)
    def randint(self, lo, hi, shape):
        return jax.random.randint(self._next(), shape, lo, hi, dtype=jnp.int32)
    def uniform(self, shape, lo=0.0, hi=1.0):
        return jax.random.uniform(self._next(), shape, jnp.bfloat16, lo, hi)
    def permutation(self, n):
        return jax.random.permutation(self._next(), n)


kernel_name = 'recurrent_scan__sliding_block_cached__moe_arch_mod__prompt'

def setup_inputs():
    _rng = _Rng(jax.random.key(int.from_bytes(__import__("os").urandom(4), "little")))
    _w = (lambda a: (lambda t: t.astype(jnp.bfloat16) if jnp.issubdtype(t.dtype, jnp.floating) else t)(jnp.asarray(a)))
    def _A_setup():
        B, Sq, D = 1, 2048, 640
        Hq, Hkv, Sk, Dh = 32, 32, 2048, 192
        assert Hq % Hkv == 0, (Hq, Hkv)
        return {
            "x": _w((lambda *s: _rng.normal(s) * 0.05)(B, Sq, D)),
            "k_cache": _w((lambda *s: _rng.normal(s) * 0.05)(B, Hkv, Sk, Dh)),
            "v_cache": _w((lambda *s: _rng.normal(s) * 0.05)(B, Hkv, Sk, Dh)),
            "wq": _w((lambda *s: _rng.normal(s) * 0.05)(D, Hq * Dh) * (D ** -0.5)),
            "wo": _w((lambda *s: _rng.normal(s) * 0.05)(Hq * Dh, D) * ((Hq * Dh) ** -0.5)),
        }
    _A_in = _A_setup()

    def _B_setup():
        B, S, D, F, C = 1, 2048, 640, 1536, 2
        return {
            "x": _w((lambda *s: _rng.normal(s) * 0.05)(B, S, D)),
            "w_r": _w((lambda *s: _rng.normal(s) * 0.05)(D)),
            "w_gate": _w((lambda *s: _rng.normal(s) * 0.05)(D, F)),
            "w_up": _w((lambda *s: _rng.normal(s) * 0.05)(D, F)),
            "w_down": _w((lambda *s: _rng.normal(s) * 0.05)(F, D)),
        }
    _B_in = _B_setup()

    return {
        "A_x": _A_in["x"],
        "A_k_cache": _A_in["k_cache"],
        "A_v_cache": _A_in["v_cache"],
        "A_wq": _A_in["wq"],
        "A_wo": _A_in["wo"],
        "B_x": _B_in["x"],
        "B_w_r": _B_in["w_r"],
        "B_w_gate": _B_in["w_gate"],
        "B_w_up": _B_in["w_up"],
        "B_w_down": _B_in["w_down"],
    }

def reference(A_x, A_k_cache, A_v_cache, A_wq, A_wo, B_x, B_w_r, B_w_gate, B_w_up, B_w_down):
    def _A_ref(x, k_cache, v_cache, wq, wo):
        B, Sq, D = x.shape
        Hq, Dh = 32, 192
        Hkv, Sk = k_cache.shape[1], k_cache.shape[2]
        W = min(4096, max(256, Sk // 4))
        rep = Hq // Hkv
        q = (lambda x, *d: x.transpose(*d))((x @ wq).reshape(B, Sq, Hq, Dh), 0, 2, 1, 3)
        k = jnp.repeat(k_cache[:, :, Sk - W:, :], rep, axis=1)
        v = jnp.repeat(v_cache[:, :, Sk - W:, :], rep, axis=1)
        scores = jnp.einsum("bhqd,bhkd->bhqk", q, k) * (Dh ** -0.5)
        p = _softmax(scores, axis=-1)
        o = jnp.einsum("bhqk,bhkd->bhqd", p, v)
        return (lambda x, *d: x.transpose(*d))(o, 0, 2, 1, 3).reshape(B, Sq, Hq * Dh) @ wo

    def _B_ref(x, w_r, w_gate, w_up, w_down):
        B, S, D = x.shape
        C = 2
        r = x @ w_r
        idx = jnp.argsort(-r, axis=-1)[:, :C]
        idx_e = jnp.repeat(idx.reshape(B, C, 1), D, axis=2)
        x_sel = jnp.take_along_axis(x, idx_e, axis=1)
        g = _silu(x_sel @ w_gate)
        u = x_sel @ w_up
        y = (g * u) @ w_down
        r_sel = _sigmoid(jnp.take_along_axis(r, idx, axis=1))
        y = y * r_sel.reshape(B, C, 1)
        b_off = (jnp.arange(B) * S).reshape(B, 1)
        flat_idx = (idx + b_off).reshape(B * C)
        zero = (x * 0.0).reshape(B * S, D)
        upd = _scatter_add(zero, flat_idx, y.reshape(B * C, D), axis=0)
        return x + upd.reshape(B, S, D)

    x = A_x
    xn = _layernorm(x, axis=-1)
    s = _A_ref(xn, A_k_cache, A_v_cache, A_wq, A_wo)
    g = _silu(_B_ref(xn, B_w_r, B_w_gate, B_w_up, B_w_down))
    return x + s * g
```

```python
import functools

import jax
import jax.numpy as jnp
import numpy as np
from jax import lax
import jax.experimental.pallas as pl
import jax.experimental.pallas.tpu as pltpu

_SQ, _D = 2048, 640
_H, _DH = 32, 192
_SK = 2048
_W = min(4096, max(256, _SK // 4))
_F = 1536
_BM = 512
_NPAIR = _H // 2
_EPS = 1e-5
_EPS_B = float(np.array([np.float32(_EPS).view(np.uint32) + 0x7FFF + ((np.float32(_EPS).view(np.uint32) >> 16) & 1)], dtype=np.uint32).__and__(np.uint32(0xFFFF0000)).view(np.float32)[0])
_QSCALE = float(_DH ** -0.5 * np.log2(np.e))

_NT = (((1,), (1,)), ((), ()))


def _layernorm_rows(x):
    xf = x.astype(jnp.float32)
    mean = jnp.mean(xf, axis=-1, keepdims=True)
    cen = xf - mean
    var = jnp.mean(cen * cen, axis=-1, keepdims=True)
    m_b = mean.astype(jnp.bfloat16).astype(jnp.float32)
    v_b = var.astype(jnp.bfloat16).astype(jnp.float32)
    den = (v_b + _EPS_B).astype(jnp.bfloat16).astype(jnp.float32)
    den = jnp.sqrt(den).astype(jnp.bfloat16).astype(jnp.float32)
    d = (xf - m_b).astype(jnp.bfloat16).astype(jnp.float32)
    return (d / den).astype(jnp.bfloat16).astype(jnp.float32)


def _kernel(x_ref, k_ref, v_ref, wq_ref, wo_ref, wr_ref, wg_hbm, wu_hbm, wd_hbm,
            o_ref,
            xq_ref, xn_ref, acc_ref, kp_ref, vp_ref, wg_ref, wu_ref, wd_ref, sems):
    step = pl.program_id(0)

    def ffn_copies():
        return (pltpu.make_async_copy(wg_hbm, wg_ref, sems.at[0]),
                pltpu.make_async_copy(wu_hbm, wu_ref, sems.at[1]),
                pltpu.make_async_copy(wd_hbm, wd_ref, sems.at[2]))

    @pl.when(step == 0)
    def _():
        for c in ffn_copies():
            c.start()

        def ln_body(i, carry):
            r0 = pl.multiple_of(i * 256, 256)
            xn = _layernorm_rows(x_ref[pl.ds(r0, 256), :])
            xn_ref[pl.ds(r0, 256), :] = xn.astype(jnp.bfloat16)
            xq_ref[pl.ds(r0, 256), :] = (xn * _QSCALE).astype(jnp.bfloat16)
            acc_ref[pl.ds(r0, 256), :] = jnp.zeros((256, _D), jnp.float32)
            return carry
        lax.fori_loop(0, _SQ // 256, ln_body, 0)

    z64 = jnp.zeros((64, _W), jnp.bfloat16)
    kp_ref[0] = jnp.concatenate([k_ref[0], z64], axis=0)
    kp_ref[1] = jnp.concatenate([z64, k_ref[1]], axis=0)
    vp_ref[0] = jnp.concatenate([v_ref[0], z64], axis=0)
    vp_ref[1] = jnp.concatenate([z64, v_ref[1]], axis=0)

    def chunk(i, carry):
        r0 = pl.multiple_of(i * _BM, _BM)
        xq = xq_ref[pl.ds(r0, _BM), :]
        q = jnp.dot(xq, wq_ref[...], preferred_element_type=jnp.float32).astype(jnp.bfloat16)
        outs = []
        for h in range(2):
            qh = q[:, 128 * h:128 * h + 256]
            s = jnp.dot(qh, kp_ref[h], preferred_element_type=jnp.float32)
            m = jnp.max(s, axis=-1, keepdims=True)
            p = jnp.exp2(s - m)
            l = jnp.sum(p, axis=-1, keepdims=True)
            o = lax.dot_general(p.astype(jnp.bfloat16), vp_ref[h], _NT, preferred_element_type=jnp.float32)
            outs.append(o * (1.0 / l))
        oa, ob = outs
        opair = jnp.concatenate([oa[:, :128], oa[:, 128:] + ob[:, :128], ob[:, 128:]], axis=1)
        acc_ref[pl.ds(r0, _BM), :] += jnp.dot(opair.astype(jnp.bfloat16), wo_ref[...],
                                              preferred_element_type=jnp.float32)
        return carry
    lax.fori_loop(0, _SQ // _BM, chunk, 0)

    @pl.when(step == _NPAIR - 1)
    def _():
        for c in ffn_copies():
            c.wait()
        xn = xn_ref[...]
        wr = wr_ref[...].astype(jnp.float32)
        r = jnp.sum(xn.astype(jnp.float32) * wr, axis=-1, keepdims=True)
        r = r.astype(jnp.bfloat16).astype(jnp.float32)
        rows = lax.broadcasted_iota(jnp.int32, (_SQ, 1), 0)
        m1 = jnp.max(r, axis=0, keepdims=True)
        i1 = jnp.min(jnp.where(r == m1, rows, _SQ), axis=0, keepdims=True)
        r2 = jnp.where(rows == i1, -jnp.inf, r)
        m2 = jnp.max(r2, axis=0, keepdims=True)
        i2 = jnp.min(jnp.where((r2 == m2) & (rows != i1), rows, _SQ), axis=0, keepdims=True)
        sel_row = lax.broadcasted_iota(jnp.int32, (16, _SQ), 0)
        sel_col = lax.broadcasted_iota(jnp.int32, (16, _SQ), 1)
        onehot = jnp.where(((sel_row == 0) & (sel_col == i1)) | ((sel_row == 1) & (sel_col == i2)),
                           1.0, 0.0).astype(jnp.bfloat16)
        xs = jnp.dot(onehot, xn, preferred_element_type=jnp.float32).astype(jnp.bfloat16)
        g = jnp.dot(xs, wg_ref[...], preferred_element_type=jnp.float32).astype(jnp.bfloat16).astype(jnp.float32)
        u = jnp.dot(xs, wu_ref[...], preferred_element_type=jnp.float32).astype(jnp.bfloat16).astype(jnp.float32)
        g = (g * jax.nn.sigmoid(g)).astype(jnp.bfloat16).astype(jnp.float32)
        hid = (g * u).astype(jnp.bfloat16)
        y = jnp.dot(hid, wd_ref[...], preferred_element_type=jnp.float32).astype(jnp.bfloat16).astype(jnp.float32)
        y1 = (y[0:1, :] * jax.nn.sigmoid(m1).astype(jnp.bfloat16).astype(jnp.float32)).astype(jnp.bfloat16).astype(jnp.float32)
        y2 = (y[1:2, :] * jax.nn.sigmoid(m2).astype(jnp.bfloat16).astype(jnp.float32)).astype(jnp.bfloat16).astype(jnp.float32)

        def fin(i, carry):
            r0 = pl.multiple_of(i * 256, 256)
            rr = r0 + lax.broadcasted_iota(jnp.int32, (256, 1), 0)
            xn_c = xn_ref[pl.ds(r0, 256), :].astype(jnp.float32)
            upd = jnp.where(rr == i1, y1, 0.0) + jnp.where(rr == i2, y2, 0.0)
            t = xn_c + upd
            gate = t * jax.nn.sigmoid(t)
            o_ref[pl.ds(r0, 256), :] = (x_ref[pl.ds(r0, 256), :].astype(jnp.float32)
                                        + acc_ref[pl.ds(r0, 256), :] * gate).astype(o_ref.dtype)
            return carry
        lax.fori_loop(0, _SQ // 256, fin, 0)


@jax.jit
def pallas_recurrent_scan__sliding_block_cached__moe_arch_mod__prompt_kernel(
    A_x, A_k_cache, A_v_cache, A_wq, A_wo, B_x, B_w_r, B_w_gate, B_w_up, B_w_down,
):
    del B_x
    x = A_x.reshape(_SQ, _D)
    k = jnp.swapaxes(A_k_cache.reshape(_H, _SK, _DH), 1, 2)
    v = jnp.swapaxes(A_v_cache.reshape(_H, _SK, _DH), 1, 2)
    wr = B_w_r.reshape(1, _D)
    nwin = _SK // _W - 1
    out = pl.pallas_call(
        _kernel,
        grid=(_NPAIR,),
        in_specs=[
            pl.BlockSpec((_SQ, _D), lambda i: (0, 0)),
            pl.BlockSpec((2, _DH, _W), lambda i: (i, 0, nwin)),
            pl.BlockSpec((2, _DH, _W), lambda i: (i, 0, nwin)),
            pl.BlockSpec((_D, 2 * _DH), lambda i: (0, i)),
            pl.BlockSpec((2 * _DH, _D), lambda i: (i, 0)),
            pl.BlockSpec((1, _D), lambda i: (0, 0)),
            pl.BlockSpec(memory_space=pl.ANY),
            pl.BlockSpec(memory_space=pl.ANY),
            pl.BlockSpec(memory_space=pl.ANY),
        ],
        out_specs=pl.BlockSpec((_SQ, _D), lambda i: (0, 0)),
        out_shape=jax.ShapeDtypeStruct((_SQ, _D), A_x.dtype),
        scratch_shapes=[
            pltpu.VMEM((_SQ, _D), jnp.bfloat16),
            pltpu.VMEM((_SQ, _D), jnp.bfloat16),
            pltpu.VMEM((_SQ, _D), jnp.float32),
            pltpu.VMEM((2, 256, _W), jnp.bfloat16),
            pltpu.VMEM((2, 256, _W), jnp.bfloat16),
            pltpu.VMEM((_D, _F), jnp.bfloat16),
            pltpu.VMEM((_D, _F), jnp.bfloat16),
            pltpu.VMEM((_F, _D), jnp.bfloat16),
            pltpu.SemaphoreType.DMA((3,)),
        ],
        compiler_params=pltpu.CompilerParams(
            dimension_semantics=("arbitrary",),
            vmem_limit_bytes=100 * 1024 * 1024,
        ),
    )(x, k, v, A_wq, A_wo, wr, B_w_gate, B_w_up, B_w_down)
    return out.reshape(1, _SQ, _D)
```

```python
import functools
import jax
import jax.numpy as jnp
import numpy as np
from jax import lax
import jax.experimental.pallas as pl
import jax.experimental.pallas.tpu as pltpu

_SQ, _D = 2048, 640
_H, _DH = 32, 192
_SK = 2048
_W = min(4096, max(256, _SK // 4))
_F = 1536
_NPAIR = _H // 2
_EPS_B = 1.0013580322265625e-05
_QSCALE = float(_DH ** -0.5 * np.log2(np.e))
_NT = (((1,), (1,)), ((), ()))
_TN = (((0,), (0,)), ((), ()))
bf16, f32 = jnp.bfloat16, jnp.float32


def _rb(x):
    return x.astype(bf16).astype(f32)


def _layernorm_rows(x):
    xf = x.astype(f32)
    mean = jnp.sum(xf, axis=-1, keepdims=True) * (1.0 / _D)
    cen = xf - mean
    var = jnp.sum(cen * cen, axis=-1, keepdims=True) * (1.0 / _D)
    return cen * lax.rsqrt(var + 1e-5)


def _silu(t):
    h = 0.5 * t
    return h * jnp.tanh(h) + h


def _kernel(x_ref, k_ref, v_ref, wq_ref, wo_ref, wr_ref, wg_hbm, wu_hbm, wd_hbm,
            o_ref,
            xq_ref, xn_ref, acc_ref, r_ref, wg_ref, wu_ref, wd_ref, sems, *, BM, mode, unroll):
    step = pl.program_id(0)

    def ffn_copies():
        return (pltpu.make_async_copy(wg_hbm, wg_ref, sems.at[0]),
                pltpu.make_async_copy(wu_hbm, wu_ref, sems.at[1]),
                pltpu.make_async_copy(wd_hbm, wd_ref, sems.at[2]))

    @pl.when(step == 0)
    def _():
        for c in ffn_copies():
            c.start()

        def ln_body(i, carry):
            r0 = pl.multiple_of(i * 256, 256)
            xnb = _layernorm_rows(x_ref[pl.ds(r0, 256), :]).astype(bf16)
            xn_ref[pl.ds(r0, 256), :] = xnb
            xn = xnb.astype(f32)
            xq_ref[pl.ds(r0, 256), :] = (xn * _QSCALE).astype(bf16)
            acc_ref[pl.ds(r0, 256), :] = jnp.zeros((256, _D), f32)
            r_ref[pl.ds(r0, 256), :] = _rb(jnp.sum(xn * wr, axis=-1, keepdims=True))
            return carry
        wr = wr_ref[...].astype(f32)
        lax.fori_loop(0, _SQ // 256, ln_body, 0)

    krow = lax.broadcasted_iota(jnp.int32, (128, _W), 0)

    def chunk(i, carry):
        r0 = pl.multiple_of(i * BM, BM)
        xq = xq_ref[pl.ds(r0, BM), :]
        q = jnp.dot(xq, wq_ref[...], preferred_element_type=f32).astype(bf16)
        kmid = k_ref[128:256, :]
        zero = jnp.zeros_like(kmid)
        ka = jnp.concatenate([k_ref[0:128, :], jnp.where(krow < 64, kmid, zero)], axis=0)
        kb = jnp.concatenate([jnp.where(krow >= 64, kmid, zero), k_ref[256:384, :]], axis=0)
        ss = [jnp.dot(q[:, 0:256], ka, preferred_element_type=f32),
              jnp.dot(q[:, 128:384], kb, preferred_element_type=f32)]
        outs = []
        for h in range(2):
            s = ss[h]
            m = jnp.max(s, axis=-1, keepdims=True)
            p = jnp.exp2(s - m)
            l = jnp.sum(p, axis=-1, keepdims=True)
            pn = (p * (1.0 / l)).astype(bf16)
            ot = lax.dot_general(v_ref[h], pn, _NT, preferred_element_type=f32)
            outs.append(ot.astype(bf16))
        ot = jnp.concatenate(outs, axis=0)
        if mode == 'tn':
            y = lax.dot_general(ot, wo_ref[...], _TN, preferred_element_type=f32)
        elif mode == 'T':
            y = jnp.dot(ot.T, wo_ref[...], preferred_element_type=f32)
        acc_ref[pl.ds(r0, BM), :] += y
        return carry
    lax.fori_loop(0, _SQ // BM, chunk, 0, unroll=unroll)

    @pl.when(step == _NPAIR - 1)
    def _():
        for c in ffn_copies():
            c.wait()
        r = r_ref[...]
        rows = lax.broadcasted_iota(jnp.int32, (_SQ, 1), 0)
        m1 = jnp.max(r, axis=0, keepdims=True)
        i1v = jnp.min(jnp.where(r == m1, rows, _SQ), axis=0, keepdims=True)
        r2 = jnp.where(rows == i1v, -jnp.inf, r)
        m2 = jnp.max(r2, axis=0, keepdims=True)
        i2v = jnp.min(jnp.where((r2 == m2) & (rows != i1v), rows, _SQ), axis=0, keepdims=True)
        i1 = i1v[0, 0]
        i2 = i2v[0, 0]
        sub = lax.broadcasted_iota(jnp.int32, (16, _D), 0)

        def take_row(i):
            base = pl.multiple_of((i // 16) * 16, 16)
            blk = xn_ref[pl.ds(base, 16), :].astype(f32)
            return jnp.sum(jnp.where(sub == i - base, blk, 0.0), axis=0, keepdims=True)
        x1 = take_row(i1)
        x2 = take_row(i2)
        xs = jnp.where(sub == 0, x1, jnp.where(sub == 1, x2, 0.0)).astype(bf16)
        g = _rb(jnp.dot(xs, wg_ref[...], preferred_element_type=f32))
        u = _rb(jnp.dot(xs, wu_ref[...], preferred_element_type=f32))
        g = _rb(_silu(g))
        hid = (g * u).astype(bf16)
        y = _rb(jnp.dot(hid, wd_ref[...], preferred_element_type=f32))
        y1 = _rb(y[0:1, :] * _rb(jax.nn.sigmoid(m1)))
        y2 = _rb(y[1:2, :] * _rb(jax.nn.sigmoid(m2)))

        def fin(i, carry):
            r0 = pl.multiple_of(i * 256, 256)
            xn_c = xn_ref[pl.ds(r0, 256), :].astype(f32)
            gate = _silu(xn_c)
            o_ref[pl.ds(r0, 256), :] = (x_ref[pl.ds(r0, 256), :].astype(f32)
                                        + acc_ref[pl.ds(r0, 256), :] * gate).astype(o_ref.dtype)
            return carry
        lax.fori_loop(0, _SQ // 256, fin, 0)

        def fix_row(i, xrow, y):
            base = pl.multiple_of((i // 16) * 16, 16)
            sl = pl.ds(base, 16)
            gate = _silu(_rb(xrow + y))
            fixed = x_ref[sl, :].astype(f32) + acc_ref[sl, :] * gate
            o_ref[sl, :] = jnp.where(sub == i - base, fixed, o_ref[sl, :].astype(f32)).astype(o_ref.dtype)
        fix_row(i1, x1, y1)
        fix_row(i2, x2, y2)


def build(BM=512, mode='tn', unroll=1):
    def fn(A_x, A_k_cache, A_v_cache, A_wq, A_wo, B_x, B_w_r, B_w_gate, B_w_up, B_w_down):
        del B_x
        x = A_x.reshape(_SQ, _D)
        k = jnp.swapaxes(A_k_cache.reshape(_H, _SK, _DH), 1, 2).reshape(_H * _DH, _SK)
        v = jnp.swapaxes(A_v_cache.reshape(_H, _SK, _DH), 1, 2)
        wr = B_w_r.reshape(1, _D)
        nwin = _SK // _W - 1
        out = pl.pallas_call(
            functools.partial(_kernel, BM=BM, mode=mode, unroll=unroll),
            grid=(_NPAIR,),
            in_specs=[
                pl.BlockSpec((_SQ, _D), lambda i: (0, 0)),
                pl.BlockSpec((2 * _DH, _W), lambda i: (i, nwin)),
                pl.BlockSpec((2, _DH, _W), lambda i: (i, 0, nwin)),
                pl.BlockSpec((_D, 2 * _DH), lambda i: (0, i)),
                pl.BlockSpec((2 * _DH, _D), lambda i: (i, 0)),
                pl.BlockSpec((1, _D), lambda i: (0, 0)),
                pl.BlockSpec(memory_space=pl.ANY),
                pl.BlockSpec(memory_space=pl.ANY),
                pl.BlockSpec(memory_space=pl.ANY),
            ],
            out_specs=pl.BlockSpec((_SQ, _D), lambda i: (0, 0)),
            out_shape=jax.ShapeDtypeStruct((_SQ, _D), A_x.dtype),
            scratch_shapes=[
                pltpu.VMEM((_SQ, _D), bf16),
                pltpu.VMEM((_SQ, _D), bf16),
                pltpu.VMEM((_SQ, _D), f32),
                pltpu.VMEM((_SQ, 1), f32),
                pltpu.VMEM((_D, _F), bf16),
                pltpu.VMEM((_D, _F), bf16),
                pltpu.VMEM((_F, _D), bf16),
                pltpu.SemaphoreType.DMA((3,)),
            ],
            compiler_params=pltpu.CompilerParams(
                dimension_semantics=("arbitrary",),
                vmem_limit_bytes=100 * 1024 * 1024,
            ),
        )(x, k, v, A_wq, A_wo, wr, B_w_gate, B_w_up, B_w_down)
        return out.reshape(1, _SQ, _D)
    return fn


_impl = build(BM=512, unroll=4)


@jax.jit
def pallas_recurrent_scan__sliding_block_cached__moe_arch_mod__prompt_kernel(
    A_x, A_k_cache, A_v_cache, A_wq, A_wo, B_x, B_w_r, B_w_gate, B_w_up, B_w_down,
):
    return _impl(A_x, A_k_cache, A_v_cache, A_wq, A_wo, B_x, B_w_r, B_w_gate, B_w_up, B_w_down)
```

```python
import functools
import jax
import jax.numpy as jnp
import numpy as np
from jax import lax
import jax.experimental.pallas as pl
import jax.experimental.pallas.tpu as pltpu

_SQ, _D = 2048, 640
_H, _DH = 32, 192
_SK = 2048
_W = min(4096, max(256, _SK // 4))
_F = 1536
_NPAIR = _H // 2
_EPS_B = 1.0013580322265625e-05
_QSCALE = float(_DH ** -0.5 * np.log2(np.e))
_NT = (((1,), (1,)), ((), ()))
_TN = (((0,), (0,)), ((), ()))
bf16, f32 = jnp.bfloat16, jnp.float32


def _rb(x):
    return x.astype(bf16).astype(f32)


def _layernorm_rows(x):
    xf = x.astype(f32)
    mean = jnp.sum(xf, axis=-1, keepdims=True) * (1.0 / _D)
    cen = xf - mean
    var = jnp.sum(cen * cen, axis=-1, keepdims=True) * (1.0 / _D)
    return cen * lax.rsqrt(var + 1e-5)


def _silu(t):
    h = 0.5 * t
    return h * jnp.tanh(h) + h


def _kernel(x_hbm, k_hbm, v_hbm, wq_hbm, wo_hbm, wr_ref, wg_hbm, wu_hbm, wd_hbm,
            o_hbm,
            x_ref, o_ref, k_buf, v_buf, wq_buf, wo_buf,
            xq_ref, xn_ref, acc_ref, r_ref, wg_ref, wu_ref, wd_ref, sems, xsem, osem, wsem, *, BM, mode, unroll):
    step = pl.program_id(0)
    NXC = 8
    XR = _SQ // NXC
    win = pl.ds(_SK - _W, _W)

    def x_copy(c):
        return pltpu.make_async_copy(x_hbm.at[pl.ds(c * XR, XR)], x_ref.at[pl.ds(c * XR, XR)], xsem.at[c])

    def o_copy(c):
        return pltpu.make_async_copy(o_ref.at[pl.ds(c * XR, XR)], o_hbm.at[pl.ds(c * XR, XR)], osem.at[c])

    def w_copies(i, slot):
        r0 = pl.multiple_of(i * (2 * _DH), 2 * _DH)
        return (pltpu.make_async_copy(k_hbm.at[pl.ds(r0, 2 * _DH), win], k_buf.at[slot], wsem.at[slot * 4 + 0]),
                pltpu.make_async_copy(v_hbm.at[pl.ds(r0, 2 * _DH), win], v_buf.at[slot], wsem.at[slot * 4 + 1]),
                pltpu.make_async_copy(wq_hbm.at[:, pl.ds(r0, 2 * _DH)], wq_buf.at[slot], wsem.at[slot * 4 + 2]),
                pltpu.make_async_copy(wo_hbm.at[pl.ds(r0, 2 * _DH), :], wo_buf.at[slot], wsem.at[slot * 4 + 3]))
    slot = step % 2

    def ffn_copies():
        return (pltpu.make_async_copy(wg_hbm, wg_ref, sems.at[0]),
                pltpu.make_async_copy(wu_hbm, wu_ref, sems.at[1]),
                pltpu.make_async_copy(wd_hbm, wd_ref, sems.at[2]))

    @pl.when(step == 0)
    def _():
        for c in range(NXC):
            x_copy(c).start()
        for cp in w_copies(0, 0):
            cp.start()

    @pl.when(step + 1 < _NPAIR)
    def _():
        for cp in w_copies(step + 1, 1 - slot):
            cp.start()

    @pl.when(step == 0)
    def _():
        for c in ffn_copies():
            c.start()

        def ln_body(i, carry):
            x_copy(i).wait()
            r0 = pl.multiple_of(i * 256, 256)
            xnb = _layernorm_rows(x_ref[pl.ds(r0, 256), :]).astype(bf16)
            xn_ref[pl.ds(r0, 256), :] = xnb
            xn = xnb.astype(f32)
            xq_ref[pl.ds(r0, 256), :] = (xn * _QSCALE).astype(bf16)
            acc_ref[pl.ds(r0, 256), :] = jnp.zeros((256, _D), f32)
            r_ref[pl.ds(r0, 256), :] = _rb(jnp.sum(xn * wr, axis=-1, keepdims=True))
            return carry
        wr = wr_ref[...].astype(f32)
        lax.fori_loop(0, _SQ // 256, ln_body, 0)

    for cp in w_copies(step, slot):
        cp.wait()
    k_ref, v_ref, wq_ref, wo_ref = k_buf.at[slot], v_buf.at[slot], wq_buf.at[slot], wo_buf.at[slot]
    krow = lax.broadcasted_iota(jnp.int32, (128, _W), 0)

    def chunk(i, carry):
        r0 = pl.multiple_of(i * BM, BM)
        xq = xq_ref[pl.ds(r0, BM), :]
        q = jnp.dot(xq, wq_ref[...], preferred_element_type=f32).astype(bf16)
        kmid = k_ref[128:256, :]
        zero = jnp.zeros_like(kmid)
        ka = jnp.concatenate([k_ref[0:128, :], jnp.where(krow < 64, kmid, zero)], axis=0)
        kb = jnp.concatenate([jnp.where(krow >= 64, kmid, zero), k_ref[256:384, :]], axis=0)
        ss = [jnp.dot(q[:, 0:256], ka, preferred_element_type=f32),
              jnp.dot(q[:, 128:384], kb, preferred_element_type=f32)]
        outs = []
        for h in range(2):
            s = ss[h]
            m = jnp.max(s, axis=-1, keepdims=True)
            p = jnp.exp2(s - m)
            l = jnp.sum(p, axis=-1, keepdims=True)
            pn = (p * (1.0 / l)).astype(bf16)
            ot = lax.dot_general(v_ref[192 * h:192 * h + 192, :], pn, _NT, preferred_element_type=f32)
            outs.append(ot.astype(bf16))
        ot = jnp.concatenate(outs, axis=0)
        if mode == 'tn':
            y = lax.dot_general(ot, wo_ref[...], _TN, preferred_element_type=f32)
        elif mode == 'T':
            y = jnp.dot(ot.T, wo_ref[...], preferred_element_type=f32)
        acc_ref[pl.ds(r0, BM), :] += y
        return carry
    lax.fori_loop(0, _SQ // BM, chunk, 0, unroll=unroll)

    @pl.when(step == _NPAIR - 1)
    def _():
        for c in ffn_copies():
            c.wait()
        r = r_ref[...]
        rows = lax.broadcasted_iota(jnp.int32, (_SQ, 1), 0)
        m1 = jnp.max(r, axis=0, keepdims=True)
        i1v = jnp.min(jnp.where(r == m1, rows, _SQ), axis=0, keepdims=True)
        r2 = jnp.where(rows == i1v, -jnp.inf, r)
        m2 = jnp.max(r2, axis=0, keepdims=True)
        i2v = jnp.min(jnp.where((r2 == m2) & (rows != i1v), rows, _SQ), axis=0, keepdims=True)
        i1 = jnp.clip(i1v[0, 0], 0, _SQ - 1)
        i2 = jnp.clip(i2v[0, 0], 0, _SQ - 1)
        sub = lax.broadcasted_iota(jnp.int32, (16, _D), 0)

        def take_row(i):
            base = pl.multiple_of((i // 16) * 16, 16)
            blk = xn_ref[pl.ds(base, 16), :].astype(f32)
            return jnp.sum(jnp.where(sub == i - base, blk, 0.0), axis=0, keepdims=True)
        x1 = take_row(i1)
        x2 = take_row(i2)
        xs = jnp.where(sub == 0, x1, jnp.where(sub == 1, x2, 0.0)).astype(bf16)
        g = _rb(jnp.dot(xs, wg_ref[...], preferred_element_type=f32))
        u = _rb(jnp.dot(xs, wu_ref[...], preferred_element_type=f32))
        g = _rb(_silu(g))
        hid = (g * u).astype(bf16)
        y = _rb(jnp.dot(hid, wd_ref[...], preferred_element_type=f32))
        y1 = _rb(y[0:1, :] * _rb(jax.nn.sigmoid(m1)))
        y2 = _rb(y[1:2, :] * _rb(jax.nn.sigmoid(m2)))

        def fix_row(i, xrow, y):
            base = pl.multiple_of((i // 16) * 16, 16)
            sl = pl.ds(base, 16)
            gate = _silu(_rb(xrow + y))
            fixed = x_ref[sl, :].astype(f32) + acc_ref[sl, :] * gate
            o_ref[sl, :] = jnp.where(sub == i - base, fixed, o_ref[sl, :].astype(f32)).astype(o_ref.dtype)

        def fin(i, carry):
            r0 = pl.multiple_of(i * 256, 256)
            xn_c = xn_ref[pl.ds(r0, 256), :].astype(f32)
            gate = _silu(xn_c)
            o_ref[pl.ds(r0, 256), :] = (x_ref[pl.ds(r0, 256), :].astype(f32)
                                        + acc_ref[pl.ds(r0, 256), :] * gate).astype(o_ref.dtype)

            @pl.when(i1 // 256 == i)
            def _():
                fix_row(i1, x1, y1)

            @pl.when(i2 // 256 == i)
            def _():
                fix_row(i2, x2, y2)
            o_copy(i).start()
            return carry
        lax.fori_loop(0, _SQ // 256, fin, 0)
        for c in range(NXC):
            o_copy(c).wait()


def build(BM=512, mode='tn', unroll=1):
    def fn(A_x, A_k_cache, A_v_cache, A_wq, A_wo, B_x, B_w_r, B_w_gate, B_w_up, B_w_down):
        del B_x
        x = A_x.reshape(_SQ, _D)
        k = jnp.swapaxes(A_k_cache.reshape(_H, _SK, _DH), 1, 2).reshape(_H * _DH, _SK)
        v = jnp.swapaxes(A_v_cache.reshape(_H, _SK, _DH), 1, 2).reshape(_H * _DH, _SK)
        wr = B_w_r.reshape(1, _D)
        nwin = _SK // _W - 1
        out = pl.pallas_call(
            functools.partial(_kernel, BM=BM, mode=mode, unroll=unroll),
            grid=(_NPAIR,),
            in_specs=[pl.BlockSpec(memory_space=pl.ANY)] * 5
            + [pl.BlockSpec((1, _D), lambda i: (0, 0))]
            + [pl.BlockSpec(memory_space=pl.ANY)] * 3,
            out_specs=pl.BlockSpec(memory_space=pl.ANY),
            out_shape=jax.ShapeDtypeStruct((_SQ, _D), A_x.dtype),
            scratch_shapes=[
                pltpu.VMEM((_SQ, _D), bf16),
                pltpu.VMEM((_SQ, _D), bf16),
                pltpu.VMEM((2, 2 * _DH, _W), bf16),
                pltpu.VMEM((2, 2 * _DH, _W), bf16),
                pltpu.VMEM((2, _D, 2 * _DH), bf16),
                pltpu.VMEM((2, 2 * _DH, _D), bf16),
                pltpu.VMEM((_SQ, _D), bf16),
                pltpu.VMEM((_SQ, _D), bf16),
                pltpu.VMEM((_SQ, _D), f32),
                pltpu.VMEM((_SQ, 1), f32),
                pltpu.VMEM((_D, _F), bf16),
                pltpu.VMEM((_D, _F), bf16),
                pltpu.VMEM((_F, _D), bf16),
                pltpu.SemaphoreType.DMA((3,)),
                pltpu.SemaphoreType.DMA((8,)),
                pltpu.SemaphoreType.DMA((8,)),
                pltpu.SemaphoreType.DMA((8,)),
            ],
            compiler_params=pltpu.CompilerParams(
                dimension_semantics=("arbitrary",),
                vmem_limit_bytes=100 * 1024 * 1024,
            ),
        )(x, k, v, A_wq, A_wo, wr, B_w_gate, B_w_up, B_w_down)
        return out.reshape(1, _SQ, _D)
    return fn


_impl = build(BM=512, unroll=4)


@jax.jit
def pallas_recurrent_scan__sliding_block_cached__moe_arch_mod__prompt_kernel(
    A_x, A_k_cache, A_v_cache, A_wq, A_wo, B_x, B_w_r, B_w_gate, B_w_up, B_w_down,
):
    return _impl(A_x, A_k_cache, A_v_cache, A_wq, A_wo, B_x, B_w_r, B_w_gate, B_w_up, B_w_down)
```
